```python
import jax
import jax.numpy as jnp

def _softmax(x, axis=-1):
    return jax.nn.softmax(x, axis=axis)

def _gelu(x):
    return jax.nn.gelu(x, approximate=True)

def _silu(x):
    return jax.nn.silu(x)

def _sigmoid(x):
    return jax.nn.sigmoid(x)

def _layernorm(x, axis=-1, eps=1e-05):
    m = jnp.mean(x, axis=axis, keepdims=True)
    v = jnp.var(x, axis=axis, keepdims=True)
    return (x - m) / jnp.sqrt(v + eps)

def _scatter_add(tgt, idx, src, axis=0):
    return tgt.at[idx].add(src)

def _segment_sum(src, seg, n):
    return jax.ops.segment_sum(src, seg, n)

class _Rng:

    def __init__(self, key):
        self._k = key

    def _next(self):
        self._k, sub = jax.random.split(self._k)
        return sub

    def normal(self, shape):
        return jax.random.normal(self._next(), shape, dtype=jnp.bfloat16)

    def randint(self, lo, hi, shape):
        return jax.random.randint(self._next(), shape, lo, hi, dtype=jnp.int32)

    def uniform(self, shape, lo=0.0, hi=1.0):
        return jax.random.uniform(self._next(), shape, jnp.bfloat16, lo, hi)

    def permutation(self, n):
        return jax.random.permutation(self._next(), n)
kernel_name = 'interleave_layers__sliding_local_dilated__mixer_gmlp__prompt'

def setup_inputs():
    _rng = _Rng(jax.random.key(int.from_bytes(__import__("os").urandom(4), "little")))
    _w = lambda a: (lambda t: t.astype(jnp.bfloat16) if jnp.issubdtype(t.dtype, jnp.floating) else t)(jnp.asarray(a))

    def _A_setup():
        B, S, D = (1, 2048, 576)
        return {'x': _w((lambda *s: _rng.normal(s) * 0.05)(B, S, D)), 'wqkv': _w((lambda *s: _rng.normal(s) * 0.05)(D, 3 * D)), 'wo': _w((lambda *s: _rng.normal(s) * 0.05)(D, D))}
    _A_in = _A_setup()

    def _B_setup():
        B, S, D, F = (1, 2048, 576, 4608)
        Fh = F // 2
        return {'x': _w((lambda *s: _rng.normal(s) * 0.05)(B, S, D)), 'w_in': _w((lambda *s: _rng.normal(s) * 0.05)(D, 2 * Fh)), 'w_sp': _w(0.01 * (lambda *s: _rng.normal(s) * 0.05)(S, S)), 'b_sp': _w(1.0 + 0.01 * (lambda *s: _rng.normal(s) * 0.05)(S)), 'w_out': _w((lambda *s: _rng.normal(s) * 0.05)(Fh, D))}
    _B_in = _B_setup()
    return {'A_x': _A_in['x'], 'A_wqkv': _A_in['wqkv'], 'A_wo': _A_in['wo'], 'B_x': _B_in['x'], 'B_w_in': _B_in['w_in'], 'B_w_sp': _B_in['w_sp'], 'B_b_sp': _B_in['b_sp'], 'B_w_out': _B_in['w_out']}

def reference(A_x, A_wqkv, A_wo, B_x, B_w_in, B_w_sp, B_b_sp, B_w_out):

    def _A_ref(x, wqkv, wo):
        B, S, D = x.shape
        H = 32
        Dh = D // H
        W, dil = (8, 2)
        qkv = (lambda x, *d: x.transpose(*d))((x @ wqkv).reshape(B, S, 3, H, Dh), 2, 0, 3, 1, 4)
        q, k, v = (qkv[0], qkv[1], qkv[2])
        scale = Dh ** (-0.5)
        pos = jnp.arange(S)
        off = jnp.arange(W) * dil
        idx = pos[:, None] - off[None, :]
        mask = idx >= 0
        idx_c = jnp.where(mask, idx, 0).reshape(-1)
        kg = k[:, :, idx_c, :].reshape(B, H, S, W, Dh)
        vg = v[:, :, idx_c, :].reshape(B, H, S, W, Dh)
        logits = jnp.einsum('bhsd,bhswd->bhsw', q, kg) * scale
        logits = jnp.where(mask[None, None, :, :], logits, -1000000000.0)
        attn = _softmax(logits, axis=-1)
        o = jnp.einsum('bhsw,bhswd->bhsd', attn, vg)
        return (lambda x, *d: x.transpose(*d))(o, 0, 2, 1, 3).reshape(B, S, D) @ wo

    def _B_ref(x, w_in, w_sp, b_sp, w_out):
        B, S, D = x.shape
        F = w_in.shape[-1]
        Fh = F // 2
        z = _gelu(jnp.einsum('bsd,df->bsf', x, w_in))
        z1 = z[..., :Fh].copy()
        z2 = _layernorm(z[..., Fh:], axis=-1)
        g = jnp.einsum('ts,bsf->btf', w_sp, z2) + b_sp[None, :, None]
        return jnp.einsum('bsf,fd->bsd', z1 * g, w_out)
    x = A_x
    x = x + _A_ref(_layernorm(x, axis=-1), A_wqkv, A_wo)
    x = x + _B_ref(_layernorm(x, axis=-1), B_w_in, B_w_sp, B_b_sp, B_w_out)
    x = x + _A_ref(_layernorm(x, axis=-1), A_wqkv, A_wo)
    x = x + _B_ref(_layernorm(x, axis=-1), B_w_in, B_w_sp, B_b_sp, B_w_out)
    return x
```

```python
import jax
import jax.numpy as jnp
from jax import lax
import jax.experimental.pallas as pl
import jax.experimental.pallas.tpu as pltpu

S, D, H, DH, FH = 2048, 576, 32, 18, 2304
TM = 256
NB = S // TM
HALO = 16
F32, BF16 = jnp.float32, jnp.bfloat16


def _dot(a, b):
    return jnp.dot(a, b, preferred_element_type=F32)


def _dot_nt(a, b):
    return lax.dot_general(a, b, (((1,), (1,)), ((), ())), preferred_element_type=F32)


def _ln(x, axis):
    m = jnp.mean(x, axis=axis, keepdims=True)
    xc = x - m
    v = jnp.mean(xc * xc, axis=axis, keepdims=True)
    return xc * lax.rsqrt(v + 1e-5)


def _gelu(x):
    c0 = 0.7978845608028654
    c1 = 0.7978845608028654 * 0.044715
    hx = 0.5 * x
    return hx * jnp.tanh(x * (c0 + c1 * (x * x))) + hx


def _kernel(x_hbm, wqkv_hbm, wo_hbm, win_hbm, wsp_hbm, b_ref, wout_hbm, o_hbm,
            xio, x32, wqkv, wqp, wo, wop, win, wsp, wout, z2n, xnb, qkv, bcol, sems):
    cp = lambda i, s, d: pltpu.make_async_copy(s, d, sems.at[i])
    copies = [cp(0, wqkv_hbm, wqkv), cp(1, x_hbm, xio), cp(2, wo_hbm, wo),
              cp(3, win_hbm, win), cp(4, wsp_hbm, wsp), cp(5, wout_hbm, wout)]
    for c in copies:
        c.start()

    def perm(nrows, ncols, row0, src_fn):
        r = lax.broadcasted_iota(jnp.int32, (nrows, ncols), 0) + row0
        c = lax.broadcasted_iota(jnp.int32, (nrows, ncols), 1)
        return jnp.where(r == src_fn(c), 1.0, 0.0).astype(BF16)

    dh = lambda c: (c & 31) * DH + (c >> 5)
    copies[0].wait()
    wqp[:, 0:512] = _dot(wqkv[:, 0:640], perm(640, 512, 0, dh)).astype(BF16)
    wqp[:, 512:1024] = _dot(wqkv[:, 512:1152], perm(640, 512, 512, lambda c: D + dh(c))).astype(BF16)
    wqp[:, 1024:1536] = _dot(wqkv[:, 1152:1728], perm(576, 512, 1152, lambda c: 2 * D + dh(c))).astype(BF16)
    wqp[:, 1536:1664] = _dot(wqkv[:, 512:1728], perm(1216, 128, 512, lambda c: D + (c >> 6) * D + 16 + dh(c & 63))).astype(BF16)
    wqp[:, 1664:1792] = _dot(wqkv[:, 0:640], perm(640, 128, 0, lambda c: jnp.where(c < 64, 16 + dh(c), -1))).astype(BF16)
    copies[2].wait()
    r = lax.broadcasted_iota(jnp.int32, (640, D), 0)
    c = lax.broadcasted_iota(jnp.int32, (640, D), 1)
    src = jnp.where(r < 512, dh(r), jnp.where(r < 576, -1, 16 + dh(r & 63)))
    wp = _dot(jnp.where(c == src, 1.0, 0.0).astype(BF16), wo[...])
    wop[...] = jnp.concatenate([wp, jnp.zeros((640, 64), F32)], 1).T[:D].astype(BF16)
    bcol[...] = jnp.broadcast_to(b_ref[...].astype(F32), (128, S)).T
    copies[1].wait()
    for i in range(NB):
        x32[i] = xio[:, i * TM:(i + 1) * TM].astype(F32)
    copies[3].wait()

    def ln_t(xt):
        xn = _ln(xt, 0)
        return jnp.concatenate([xn, jnp.zeros((64, TM), F32)], 0).T[:, :D].astype(BF16)

    def stage_a(i):
        qkv[HALO + i * TM:HALO + (i + 1) * TM, :] = _dot(ln_t(x32[i]), wqp[...])
        if i == 0:
            qkv[0:HALO, :] = jnp.broadcast_to(qkv[HALO:HALO + 1, :], (HALO, 1792))

    def stage_b(i):
        r0 = HALO + i * TM
        q = [qkv[r0:r0 + TM, j * 128:(j + 1) * 128] for j in (0, 1, 2, 3, 13)]
        sh = [qkv[r0 - 8 - s:r0 + TM - s, 512:1664] for s in (0, 2, 4, 6)]
        win_ = lambda w: sh[w % 4][8:] if w < 4 else sh[w % 4][:TM]
        lg = []
        for w in range(8):
            k = win_(w)
            p = q[4] * k[:, 1024:1152]
            for j in range(4):
                p = p + q[j] * k[:, j * 128:(j + 1) * 128]
            p = p + pltpu.roll(p, 64, 1)
            p = p + pltpu.roll(p, 32, 1)
            p = p * (DH ** -0.5)
            if i == 0:
                p = jnp.where(lax.broadcasted_iota(jnp.int32, (TM, 128), 0) >= 2 * w, p, -1e9)
            lg.append(p)
        mx = lg[0]
        for w in range(1, 8):
            mx = jnp.maximum(mx, lg[w])
        e = [jnp.exp(t - mx) for t in lg]
        den = e[0]
        for w in range(1, 8):
            den = den + e[w]
        inv = 1.0 / den
        o = []
        for j in range(5):
            acc = None
            for w in range(8):
                t = e[w] * win_(w)[:, 512 + j * 128:640 + j * 128]
                acc = t if acc is None else acc + t
            o.append((acc * inv).astype(BF16))
        x = x32[i] + _dot_nt(wop[...], jnp.concatenate(o, axis=1))
        x32[i] = x
        xnb[i] = ln_t(x)

    def stage_c(i):
        z2n[i * TM:(i + 1) * TM, :] = _ln(_gelu(_dot(xnb[i], win[:, FH:])), -1).astype(BF16)

    def layer(l, _):
        with jax.named_scope("p1"):
            for j in range(NB + 2):
                if j < NB:
                    stage_a(j)
                if 0 <= j - 1 < NB:
                    stage_b(j - 1)
                if 0 <= j - 2 < NB:
                    stage_c(j - 2)

        @pl.when(l == 0)
        def _():
            copies[4].wait()
            copies[5].wait()

        def phase2(i, _):
            rows = pl.ds(pl.multiple_of(i * TM, TM), TM)
            xn = xnb[i]
            ws = wsp[rows, :]
            bc = bcol[rows, :]
            acc = x32[i]
            FC = 768
            for c in range(FH // FC):
                g = _dot(ws, z2n[:, c * FC:(c + 1) * FC])
                z1 = _gelu(_dot(xn, win[:, c * FC:(c + 1) * FC]))
                h = (z1 * (g + jnp.tile(bc, (1, FC // 128)))).astype(BF16)
                acc = acc + _dot_nt(wout[:, c * FC:(c + 1) * FC], h)
            x32[i] = acc

        with jax.named_scope("p2"):
            lax.fori_loop(0, NB, phase2, None)

    lax.fori_loop(0, 2, layer, None)
    for i in range(NB):
        xio[:, i * TM:(i + 1) * TM] = x32[i].astype(BF16)
    oc = cp(6, xio, o_hbm)
    oc.start()
    oc.wait()


@jax.jit
def pallas_interleave_layers__sliding_local_dilated__mixer_gmlp__prompt_kernel(
    A_x, A_wqkv, A_wo, B_x, B_w_in, B_w_sp, B_b_sp, B_w_out,
):
    del B_x
    hbm = pl.BlockSpec(memory_space=pltpu.HBM)
    out = pl.pallas_call(
        _kernel,
        in_specs=[hbm, hbm, hbm, hbm, hbm, pl.BlockSpec(memory_space=pltpu.VMEM), hbm],
        out_specs=hbm,
        out_shape=jax.ShapeDtypeStruct((D, S), BF16),
        scratch_shapes=[
            pltpu.VMEM((D, S), BF16), pltpu.VMEM((NB, D, TM), F32),
            pltpu.VMEM((D, 3 * D), BF16), pltpu.VMEM((D, 1792), BF16),
            pltpu.VMEM((D, D), BF16), pltpu.VMEM((D, 640), BF16),
            pltpu.VMEM((D, 2 * FH), BF16), pltpu.VMEM((S, S), BF16), pltpu.VMEM((D, FH), BF16),
            pltpu.VMEM((S, FH), BF16), pltpu.VMEM((NB, TM, D), BF16),
            pltpu.VMEM((S + HALO, 1792), F32), pltpu.VMEM((S, 128), F32),
            pltpu.SemaphoreType.DMA((7,)),
        ],
        compiler_params=pltpu.CompilerParams(vmem_limit_bytes=100 * 1024 * 1024),
    )(A_x.reshape(S, D).T, A_wqkv, A_wo, B_w_in, B_w_sp, B_b_sp.reshape(1, S), B_w_out.T)
    return out.T.reshape(1, S, D)
```

```python
import jax
import jax.numpy as jnp
from jax import lax
import jax.experimental.pallas as pl
import jax.experimental.pallas.tpu as pltpu

S, D, H, DH, FH = 2048, 576, 32, 18, 2304
TM = 256
NB = S // TM
HALO = 16
RC = 32
ZC = 512
F32, BF16 = jnp.float32, jnp.bfloat16


def _dot(a, b):
    return jnp.dot(a, b, preferred_element_type=F32)


def _dot_nt(a, b):
    return lax.dot_general(a, b, (((1,), (1,)), ((), ())), preferred_element_type=F32)


def _ln(x, axis):
    m = jnp.mean(x, axis=axis, keepdims=True)
    xc = x - m
    v = jnp.mean(xc * xc, axis=axis, keepdims=True)
    return xc * lax.rsqrt(v + 1e-5)


def _gelu(x):
    c0 = 0.7978845608028654
    c1 = 0.7978845608028654 * 0.044715
    hx = 0.5 * x
    return hx * jnp.tanh(x * (c0 + c1 * (x * x))) + hx


def _kernel(x_hbm, wqkv_hbm, wo_hbm, win_hbm, wsp_hbm, b_ref, wout_hbm, o_hbm,
            xio, x32, wqkv, wqp, wo, wop, win, wsp, wout, z2n, xnb, qkv, bcol, wt, ob, zt, sems):
    cp = lambda i, s, d: pltpu.make_async_copy(s, d, sems.at[i])
    copies = [cp(0, wqkv_hbm, wqkv), cp(1, x_hbm, xio), cp(2, wo_hbm, wo),
              cp(3, win_hbm, win), cp(4, wsp_hbm, wsp), cp(5, wout_hbm, wout)]
    for i in (0, 2, 1):
        copies[i].start()
    bcol[...] = jnp.broadcast_to(b_ref[...].astype(F32), (128, S)).T
    copies[0].wait()
    copies[3].start()

    w = jnp.concatenate([wqkv[...].astype(F32), jnp.zeros((D, 64), F32)], 1)
    w = jnp.concatenate([w, jnp.zeros((64, 1792), F32)], 0).T
    for j in range(5):
        wt[j] = w[:, j * 128:(j + 1) * 128]

    def heads(r0):
        return jnp.concatenate([wt[j, pl.ds(r0, H, stride=DH), :] for j in range(5)], 1)

    for d in range(16):
        for t in range(3):
            wqp[t * 512 + d * H:t * 512 + (d + 1) * H, :] = heads(t * D + d)[:, :D].astype(BF16)
    for n, t in enumerate((1, 2, 0)):
        for d in range(2):
            r = 1536 + n * 64 + d * H
            wqp[r:r + H, :] = heads(t * D + 16 + d)[:, :D].astype(BF16)
    wqp[1728:, :] = jnp.zeros((64, D), BF16)
    copies[2].wait()
    w = jnp.concatenate([wo[...].astype(F32), jnp.zeros((D, 64), F32)], 1)
    for j in range(5):
        wt[j, 0:D, :] = w[:, j * 128:(j + 1) * 128]
    wp = [heads(d) for d in range(16)] + [jnp.zeros((64, 640), F32), heads(16), heads(17)]
    wop[...] = jnp.concatenate(wp, 0).T[:D].astype(BF16)
    copies[1].wait()
    copies[4].start()
    copies[5].start()
    for i in range(NB):
        x32[i] = xio[:, i * TM:(i + 1) * TM].astype(F32)

    def ln_t(xt):
        xn = _ln(xt, 0)
        return jnp.concatenate([xn, jnp.zeros((64, TM), F32)], 0).T[:, :D].astype(BF16)

    def stage_a(i):
        xnb[i] = ln_t(x32[i])
        yield

    def stage_q(i):
        for c0, c1 in ((0, 512), (512, 1024), (1024, 1536), (1536, 1792)):
            t = _dot_nt(xnb[i], wqp[c0:c1, :])
            for c in range(c0, c1, 128):
                qkv[c // 128, HALO + i * TM:HALO + (i + 1) * TM, :] = t[:, c - c0:c - c0 + 128]
            yield
        if i == 0:
            for c in range(4, 13):
                qkv[c, 0:HALO, :] = jnp.broadcast_to(qkv[c, HALO:HALO + 1, :], (HALO, 128))

    def stage_b(i):
        for rc in range(TM // RC):
            r0 = HALO + i * TM + rc * RC

            def win_(c0, s):
                t = qkv[c0 // 128, r0 - 8 - s:r0 + RC - s, :]
                return t[8:], t[:RC]

            lg = [None] * 8
            for cq, ck in ((1664, 1536), (0, 512), (128, 640), (256, 768), (384, 896)):
                q = qkv[cq // 128, r0:r0 + RC, :]
                for s in range(4):
                    for w, k in zip((s, s + 4), win_(ck, 2 * s)):
                        lg[w] = q * k if lg[w] is None else lg[w] + q * k
            for w in range(8):
                p = lg[w]
                p = p + pltpu.roll(p, 64, 1)
                p = p + pltpu.roll(p, 32, 1)
                p = p * (DH ** -0.5)
                if i == 0 and rc == 0:
                    p = jnp.where(lax.broadcasted_iota(jnp.int32, (RC, 128), 0) >= 2 * w, p, -1e9)
                lg[w] = p
            mx = lg[0]
            for w in range(1, 8):
                mx = jnp.maximum(mx, lg[w])
            e = [jnp.exp(t - mx) for t in lg]
            den = e[0]
            for w in range(1, 8):
                den = den + e[w]
            inv = 1.0 / den
            for j in range(5):
                acc = None
                for s in range(4):
                    for w, v in zip((s, s + 4), win_(1024 + j * 128, 2 * s)):
                        acc = e[w] * v if acc is None else acc + e[w] * v
                ob[i % 2, rc * RC:(rc + 1) * RC, j * 128:(j + 1) * 128] = (acc * inv).astype(BF16)
            yield

    def stage_o(i):
        x = x32[i] + _dot_nt(wop[...], ob[i % 2])
        x32[i] = x
        yield
        xnb[i] = ln_t(x)
        yield

    def stage_c(i):
        for c0 in range(0, FH, ZC):
            c1 = min(c0 + ZC, FH)
            zt[i % 2, :, c0:c1] = _gelu(_dot(xnb[i], win[:, FH + c0:FH + c1]))
            yield

    def stage_d(i):
        for r in range(0, TM, RC):
            z2n[i * TM + r:i * TM + r + RC, :] = _ln(zt[i % 2, r:r + RC, :], -1).astype(BF16)
            yield

    stages = (stage_a, stage_q, stage_b, stage_o, stage_c, stage_d)

    def layer(l, _):
        with jax.named_scope("p1"):
            for j in range(NB + len(stages) - 1):
                if j == 4:
                    pl.when(l == 0)(copies[3].wait)
                gens = [st(j - k) for k, st in enumerate(stages) if 0 <= j - k < NB]
                while gens:
                    gens = [g for g in gens if next(g, 0) is None]

        @pl.when(l == 0)
        def _():
            copies[4].wait()
            copies[5].wait()

        def phase2(i, _):
            rows = pl.ds(pl.multiple_of(i * TM, TM), TM)
            xn = xnb[i]
            ws = wsp[rows, :]
            bc = bcol[rows, :]
            acc = x32[i]
            FC = 768
            for c in range(FH // FC):
                g = _dot(ws, z2n[:, c * FC:(c + 1) * FC])
                z1 = _gelu(_dot(xn, win[:, c * FC:(c + 1) * FC]))
                h = (z1 * (g + jnp.tile(bc, (1, FC // 128)))).astype(BF16)
                acc = acc + _dot_nt(wout[:, c * FC:(c + 1) * FC], h)
            x32[i] = acc

            @pl.when(l == 1)
            def _():
                xio[:, rows] = acc.astype(BF16)
                cp(6 + i, xio.at[:, rows], o_hbm.at[:, rows]).start()

        with jax.named_scope("p2"):
            lax.fori_loop(0, NB, phase2, None)

    lax.fori_loop(0, 2, layer, None)
    for i in range(NB):
        rows = pl.ds(i * TM, TM)
        cp(6 + i, xio.at[:, rows], o_hbm.at[:, rows]).wait()


@jax.jit
def pallas_interleave_layers__sliding_local_dilated__mixer_gmlp__prompt_kernel(
    A_x, A_wqkv, A_wo, B_x, B_w_in, B_w_sp, B_b_sp, B_w_out,
):
    del B_x
    hbm = pl.BlockSpec(memory_space=pltpu.HBM)
    out = pl.pallas_call(
        _kernel,
        in_specs=[hbm, hbm, hbm, hbm, hbm, pl.BlockSpec(memory_space=pltpu.VMEM), hbm],
        out_specs=hbm,
        out_shape=jax.ShapeDtypeStruct((D, S), BF16),
        scratch_shapes=[
            pltpu.VMEM((D, S), BF16), pltpu.VMEM((NB, D, TM), F32),
            pltpu.VMEM((D, 3 * D), BF16), pltpu.VMEM((1792, D), BF16),
            pltpu.VMEM((D, D), BF16), pltpu.VMEM((D, 640), BF16),
            pltpu.VMEM((D, 2 * FH), BF16), pltpu.VMEM((S, S), BF16), pltpu.VMEM((D, FH), BF16),
            pltpu.VMEM((S, FH), BF16), pltpu.VMEM((NB, TM, D), BF16),
            pltpu.VMEM((14, S + HALO, 128), F32), pltpu.VMEM((S, 128), F32),
            pltpu.VMEM((5, 1792, 128), F32), pltpu.VMEM((2, TM, 640), BF16), pltpu.VMEM((2, TM, FH), F32),
            pltpu.SemaphoreType.DMA((6 + NB,)),
        ],
        compiler_params=pltpu.CompilerParams(vmem_limit_bytes=100 * 1024 * 1024),
    )(A_x.reshape(S, D).T, A_wqkv, A_wo, B_w_in, B_w_sp, B_b_sp.reshape(1, S), B_w_out.T)
    return out.T.reshape(1, S, D)
```

```python
import jax
import jax.numpy as jnp
from jax import lax
import jax.experimental.pallas as pl
import jax.experimental.pallas.tpu as pltpu

S, D, H, DH, FH = 2048, 576, 32, 18, 2304
TM = 256
NB = S // TM
HALO = 16
SCHED = "a0,q0,a1,a2 q1,q2,b0,a3 q3,b1,o0,a4 q4,b2,o1,c0,a5 q5,b3,o2,c1,d0,a6 q6,b4,o3,c2,d1,a7 q7,b5,o4,c3,d2 b6,o5,c4,d3 b7,o6,c5,d4 o7,c6,d5 c7,d6 d7"
ORD='aocbqd'
ZC = 512
F32, BF16 = jnp.float32, jnp.bfloat16


def _dot(a, b):
    return jnp.dot(a, b, preferred_element_type=F32)


def _dot_nt(a, b):
    return lax.dot_general(a, b, (((1,), (1,)), ((), ())), preferred_element_type=F32)


def _ln(x, axis):
    m = jnp.mean(x, axis=axis, keepdims=True)
    xc = x - m
    v = jnp.mean(xc * xc, axis=axis, keepdims=True)
    return xc * lax.rsqrt(v + 1e-5)


def _gelu(x):
    c0 = 0.7978845608028654
    c1 = 0.7978845608028654 * 0.044715
    hx = 0.5 * x
    return hx * jnp.tanh(x * (c0 + c1 * (x * x))) + hx


def _kernel(x_hbm, wqkv_hbm, wo_hbm, win_hbm, wsp_hbm, b_ref, wout_hbm, o_hbm,
            xio, x32, wqkv, wqp, wo, wop, win, wsp, wout, z2n, xnb, qkv, bcol, wt, ob, zt, sems):
    cp = lambda i, s, d: pltpu.make_async_copy(s, d, sems.at[i])
    copies = [cp(0, wqkv_hbm, wqkv), cp(1, x_hbm, xio), cp(2, wo_hbm, wo),
              cp(3, win_hbm, win), cp(4, wsp_hbm, wsp), cp(5, wout_hbm, wout)]
    for i in (0, 2, 1):
        copies[i].start()
    bcol[...] = jnp.broadcast_to(b_ref[...].astype(F32), (128, S)).T
    copies[0].wait()
    copies[3].start()

    w = jnp.concatenate([wqkv[...].astype(F32), jnp.zeros((D, 64), F32)], 1)
    w = jnp.concatenate([w, jnp.zeros((64, 1792), F32)], 0).T
    for j in range(5):
        wt[j] = w[:, j * 128:(j + 1) * 128]

    def heads(r0):
        return jnp.concatenate([wt[j, pl.ds(r0, H, stride=DH), :] for j in range(5)], 1)

    for d in range(16):
        for t in range(3):
            wqp[t * 512 + d * H:t * 512 + (d + 1) * H, :] = heads(t * D + d)[:, :D].astype(BF16)
    for n, t in enumerate((1, 2, 0)):
        for d in range(2):
            r = 1536 + n * 64 + d * H
            wqp[r:r + H, :] = heads(t * D + 16 + d)[:, :D].astype(BF16)
    wqp[1728:, :] = jnp.zeros((64, D), BF16)
    copies[2].wait()
    w = jnp.concatenate([wo[...].astype(F32), jnp.zeros((D, 64), F32)], 1)
    for j in range(5):
        wt[j, 0:D, :] = w[:, j * 128:(j + 1) * 128]
    wp = [heads(d) for d in range(16)] + [jnp.zeros((64, 640), F32), heads(16), heads(17)]
    wop[...] = jnp.concatenate(wp, 0).T[:D].astype(BF16)
    copies[1].wait()
    copies[4].start()
    copies[5].start()
    for i in range(NB):
        x32[i] = xio[:, i * TM:(i + 1) * TM].astype(F32)

    def ln_t(xt):
        xn = _ln(xt, 0)
        return jnp.concatenate([xn, jnp.zeros((64, TM), F32)], 0).T[:, :D].astype(BF16)

    def stage_a(i):
        xnb[i] = ln_t(x32[i])
        yield

    def stage_q(i):
        for c0, c1 in [(c, c + 256) for c in range(0, 1792, 256)]:
            t = _dot_nt(xnb[i], wqp[c0:c1, :])
            for c in range(c0, c1, 128):
                qkv[c // 128, HALO + i * TM:HALO + (i + 1) * TM, :] = t[:, c - c0:c - c0 + 128]
            yield
        if i == 0:
            for c in range(4, 13):
                qkv[c, 0:HALO, :] = jnp.broadcast_to(qkv[c, HALO:HALO + 1, :], (HALO, 128))

    def stage_b(i):
        RC = 64 if i in (1, 6, 7) else 16
        for rc in range(TM // RC):
            r0 = HALO + i * TM + rc * RC

            def win_(c0, s):
                t = qkv[c0 // 128, r0 - 8 - s:r0 + RC - s, :]
                return t[8:], t[:RC]

            lg = [None] * 8
            for cq, ck in ((1664, 1536), (0, 512), (128, 640), (256, 768), (384, 896)):
                q = qkv[cq // 128, r0:r0 + RC, :]
                for s in range(4):
                    for w, k in zip((s, s + 4), win_(ck, 2 * s)):
                        lg[w] = q * k if lg[w] is None else lg[w] + q * k
            for w in range(8):
                p = lg[w]
                p = p + pltpu.roll(p, 64, 1)
                p = p + pltpu.roll(p, 32, 1)
                p = p * (DH ** -0.5)
                if i == 0 and rc == 0:
                    p = jnp.where(lax.broadcasted_iota(jnp.int32, (RC, 128), 0) >= 2 * w, p, -1e9)
                lg[w] = p
            mx = lg[0]
            for w in range(1, 8):
                mx = jnp.maximum(mx, lg[w])
            e = [jnp.exp(t - mx) for t in lg]
            den = e[0]
            for w in range(1, 8):
                den = den + e[w]
            inv = 1.0 / den
            for j in range(5):
                acc = None
                for s in range(4):
                    for w, v in zip((s, s + 4), win_(1024 + j * 128, 2 * s)):
                        acc = e[w] * v if acc is None else acc + e[w] * v
                ob[i % 2, rc * RC:(rc + 1) * RC, j * 128:(j + 1) * 128] = (acc * inv).astype(BF16)
            yield

    def stage_o(i):
        x = x32[i] + _dot_nt(wop[...], ob[i % 2])
        x32[i] = x
        yield
        xnb[i] = ln_t(x)
        yield

    def stage_c(i):
        for c0 in range(0, FH, ZC):
            c1 = min(c0 + ZC, FH)
            zt[i % 2, :, c0:c1] = _gelu(_dot(xnb[i], win[:, FH + c0:FH + c1]))
            yield

    def stage_d(i):
        for r in range(0, TM, 16):
            z2n[i * TM + r:i * TM + r + 16, :] = _ln(zt[i % 2, r:r + 16, :], -1).astype(BF16)
            yield

    stages = dict(a=stage_a, q=stage_q, b=stage_b, o=stage_o, c=stage_c, d=stage_d)

    def layer(l, _):
        with jax.named_scope("p1"):
            for j, step in enumerate(SCHED.split()):
                if 'c0' in step:
                    pl.when(l == 0)(copies[3].wait)

                @pl.when(l != 7 + j)
                @jax.named_scope(step.replace(',',''))
                def _():
                    gens = [stages[t[0]](int(t[1])) for t in sorted(step.split(','), key=lambda t: ORD.index(t[0])) if j]  or [stages[t[0]](int(t[1])) for t in step.split(',')]
                    while gens:
                        gens = [g for g in gens if next(g, 0) is None]

        @pl.when(l == 0)
        def _():
            copies[4].wait()
            copies[5].wait()

        def phase2(i, _):
            rows = pl.ds(pl.multiple_of(i * TM, TM), TM)
            xn = xnb[i]
            ws = wsp[rows, :]
            bc = bcol[rows, :]
            acc = x32[i]
            FC = 768
            for c in range(FH // FC):
                g = _dot(ws, z2n[:, c * FC:(c + 1) * FC])
                z1 = _gelu(_dot(xn, win[:, c * FC:(c + 1) * FC]))
                h = (z1 * (g + jnp.tile(bc, (1, FC // 128)))).astype(BF16)
                acc = acc + _dot_nt(wout[:, c * FC:(c + 1) * FC], h)
            x32[i] = acc

            @pl.when(l == 1)
            def _():
                xio[:, rows] = acc.astype(BF16)
                cp(6 + i, xio.at[:, rows], o_hbm.at[:, rows]).start()

        with jax.named_scope("p2"):
            lax.fori_loop(0, NB, phase2, None)

    lax.fori_loop(0, 2, layer, None)
    for i in range(NB):
        rows = pl.ds(i * TM, TM)
        cp(6 + i, xio.at[:, rows], o_hbm.at[:, rows]).wait()


@jax.jit
def pallas_interleave_layers__sliding_local_dilated__mixer_gmlp__prompt_kernel(
    A_x, A_wqkv, A_wo, B_x, B_w_in, B_w_sp, B_b_sp, B_w_out,
):
    del B_x
    hbm = pl.BlockSpec(memory_space=pltpu.HBM)
    out = pl.pallas_call(
        _kernel,
        in_specs=[hbm, hbm, hbm, hbm, hbm, pl.BlockSpec(memory_space=pltpu.VMEM), hbm],
        out_specs=hbm,
        out_shape=jax.ShapeDtypeStruct((D, S), BF16),
        scratch_shapes=[
            pltpu.VMEM((D, S), BF16), pltpu.VMEM((NB, D, TM), F32),
            pltpu.VMEM((D, 3 * D), BF16), pltpu.VMEM((1792, D), BF16),
            pltpu.VMEM((D, D), BF16), pltpu.VMEM((D, 640), BF16),
            pltpu.VMEM((D, 2 * FH), BF16), pltpu.VMEM((S, S), BF16), pltpu.VMEM((D, FH), BF16),
            pltpu.VMEM((S, FH), BF16), pltpu.VMEM((NB, TM, D), BF16),
            pltpu.VMEM((14, S + HALO, 128), F32), pltpu.VMEM((S, 128), F32),
            pltpu.VMEM((5, 1792, 128), F32), pltpu.VMEM((2, TM, 640), BF16), pltpu.VMEM((2, TM, FH), F32),
            pltpu.SemaphoreType.DMA((6 + NB,)),
        ],
        compiler_params=pltpu.CompilerParams(vmem_limit_bytes=100 * 1024 * 1024),
    )(A_x.reshape(S, D).T, A_wqkv, A_wo, B_w_in, B_w_sp, B_b_sp.reshape(1, S), B_w_out.T)
    return out.T.reshape(1, S, D)
```

```python
import jax
import jax.numpy as jnp
from jax import lax
import jax.experimental.pallas as pl
import jax.experimental.pallas.tpu as pltpu

S, D, H, DH, FH = 2048, 576, 32, 18, 2304
TM = 256
NB = S // TM
HALO = 16
SCHED = "a0,q0,a1,a2 q1,q2,b0,a3 q3,b1,o0,a4 q4,b2,o1,c0,a5 q5,b3,o2,c1,d0,a6 q6,b4,o3,c2,d1,a7 q7,b5,o4,c3,d2 b6,o5,c4,d3 b7,o6,c5,d4 o7,c6,d5 c7,d6 d7"
ORD='aocbqd'
ZC = 512
F32, BF16 = jnp.float32, jnp.bfloat16


def _dot(a, b):
    return jnp.dot(a, b, preferred_element_type=F32)


def _dot_nt(a, b):
    return lax.dot_general(a, b, (((1,), (1,)), ((), ())), preferred_element_type=F32)


def _ln(x, axis):
    m = jnp.mean(x, axis=axis, keepdims=True)
    xc = x - m
    v = jnp.mean(xc * xc, axis=axis, keepdims=True)
    return xc * lax.rsqrt(v + 1e-5)


def _gelu(x):
    c0 = 0.7978845608028654
    c1 = 0.7978845608028654 * 0.044715
    hx = 0.5 * x
    return hx * jnp.tanh(x * (c0 + c1 * (x * x))) + hx


def _kernel(x_hbm, wqkv_hbm, wo_hbm, win_hbm, wsp_hbm, b_ref, wout_hbm, o_hbm,
            xio, x32, wqkv, wqp, wo, wop, win, wsp, wout, z2n, xnb, qkv, bcol, wt, ob, zt, z1p, sems):
    cp = lambda i, s, d: pltpu.make_async_copy(s, d, sems.at[i])
    copies = [cp(0, wqkv_hbm, wqkv), cp(1, x_hbm, xio), cp(2, wo_hbm, wo),
              cp(3, win_hbm, win), cp(4, wsp_hbm, wsp), cp(5, wout_hbm, wout)]
    for i in (0, 2, 1):
        copies[i].start()
    bcol[...] = jnp.broadcast_to(b_ref[...].astype(F32), (128, S)).T
    copies[0].wait()
    copies[3].start()

    w = jnp.concatenate([wqkv[...].astype(F32), jnp.zeros((D, 64), F32)], 1)
    w = jnp.concatenate([w, jnp.zeros((64, 1792), F32)], 0).T
    for j in range(5):
        wt[j] = w[:, j * 128:(j + 1) * 128]

    def heads(r0):
        return jnp.concatenate([wt[j, pl.ds(r0, H, stride=DH), :] for j in range(5)], 1)

    for d in range(16):
        for t in range(3):
            wqp[t * 512 + d * H:t * 512 + (d + 1) * H, :] = heads(t * D + d)[:, :D].astype(BF16)
    for n, t in enumerate((1, 2, 0)):
        for d in range(2):
            r = 1536 + n * 64 + d * H
            wqp[r:r + H, :] = heads(t * D + 16 + d)[:, :D].astype(BF16)
    wqp[1728:, :] = jnp.zeros((64, D), BF16)
    copies[2].wait()
    w = jnp.concatenate([wo[...].astype(F32), jnp.zeros((D, 64), F32)], 1)
    for j in range(5):
        wt[j, 0:D, :] = w[:, j * 128:(j + 1) * 128]
    wp = [heads(d) for d in range(16)] + [jnp.zeros((64, 640), F32), heads(16), heads(17)]
    wop[...] = jnp.concatenate(wp, 0).T[:D].astype(BF16)
    copies[1].wait()
    copies[4].start()
    copies[5].start()
    for i in range(NB):
        x32[i] = xio[:, i * TM:(i + 1) * TM].astype(F32)

    def ln_t(xt):
        xn = _ln(xt, 0)
        return jnp.concatenate([xn, jnp.zeros((64, TM), F32)], 0).T[:, :D].astype(BF16)

    def stage_a(i):
        xnb[i] = ln_t(x32[i])
        yield

    def stage_q(i):
        for c0, c1 in [(c, c + 256) for c in range(0, 1792, 256)]:
            t = _dot_nt(xnb[i], wqp[c0:c1, :])
            for c in range(c0, c1, 128):
                qkv[c // 128, HALO + i * TM:HALO + (i + 1) * TM, :] = t[:, c - c0:c - c0 + 128]
            yield
        if i == 0:
            for c in range(4, 13):
                qkv[c, 0:HALO, :] = jnp.broadcast_to(qkv[c, HALO:HALO + 1, :], (HALO, 128))

    def stage_b(i):
        RC = 64 if i in (1,) else 16
        for rc in range(TM // RC):
            r0 = HALO + i * TM + rc * RC

            def win_(c0, s):
                t = qkv[c0 // 128, r0 - 8 - s:r0 + RC - s, :]
                return t[8:], t[:RC]

            lg = [None] * 8
            for cq, ck in ((1664, 1536), (0, 512), (128, 640), (256, 768), (384, 896)):
                q = qkv[cq // 128, r0:r0 + RC, :]
                for s in range(4):
                    for w, k in zip((s, s + 4), win_(ck, 2 * s)):
                        lg[w] = q * k if lg[w] is None else lg[w] + q * k
            for w in range(8):
                p = lg[w]
                p = p + pltpu.roll(p, 64, 1)
                p = p + pltpu.roll(p, 32, 1)
                p = p * (DH ** -0.5)
                if i == 0 and rc == 0:
                    p = jnp.where(lax.broadcasted_iota(jnp.int32, (RC, 128), 0) >= 2 * w, p, -1e9)
                lg[w] = p
            mx = lg[0]
            for w in range(1, 8):
                mx = jnp.maximum(mx, lg[w])
            e = [jnp.exp(t - mx) for t in lg]
            den = e[0]
            for w in range(1, 8):
                den = den + e[w]
            inv = 1.0 / den
            for j in range(5):
                acc = None
                for s in range(4):
                    for w, v in zip((s, s + 4), win_(1024 + j * 128, 2 * s)):
                        acc = e[w] * v if acc is None else acc + e[w] * v
                ob[i % 2, rc * RC:(rc + 1) * RC, j * 128:(j + 1) * 128] = (acc * inv).astype(BF16)
            yield

    def stage_o(i):
        x = x32[i] + _dot_nt(wop[...], ob[i % 2])
        x32[i] = x
        yield
        xnb[i] = ln_t(x)
        yield

    def stage_c(i):
        for c0 in range(0, FH, ZC):
            c1 = min(c0 + ZC, FH)
            zt[i % 2, :, c0:c1] = _gelu(_dot(xnb[i], win[:, FH + c0:FH + c1]))
            yield
            z1p[i, :, c0:c1] = _dot(xnb[i], win[:, c0:c1])
            yield

    def stage_d(i):
        for r in range(0, TM, 16):
            z2n[i * TM + r:i * TM + r + 16, :] = _ln(zt[i % 2, r:r + 16, :], -1).astype(BF16)
            yield

    stages = dict(a=stage_a, q=stage_q, b=stage_b, o=stage_o, c=stage_c, d=stage_d)

    def layer(l, _):
        with jax.named_scope("p1"):
            for j, step in enumerate(SCHED.split()):
                if 'c0' in step:
                    pl.when(l == 0)(copies[3].wait)

                @pl.when(l != 7 + j)
                @jax.named_scope(step.replace(',',''))
                def _():
                    gens = [stages[t[0]](int(t[1])) for t in sorted(step.split(','), key=lambda t: ORD.index(t[0])) if j]  or [stages[t[0]](int(t[1])) for t in step.split(',')]
                    while gens:
                        gens = [g for g in gens if next(g, 0) is None]

        @pl.when(l == 0)
        def _():
            copies[4].wait()
            copies[5].wait()

        def phase2(i, _):
            rows = pl.ds(pl.multiple_of(i * TM, TM), TM)
            ws = wsp[rows, :]
            bc = bcol[rows, :]
            acc = x32[i]
            FC = 768
            for c in range(FH // FC):
                g = _dot(ws, z2n[:, c * FC:(c + 1) * FC])
                z1 = _gelu(z1p[i, :, c * FC:(c + 1) * FC])
                h = (z1 * (g + jnp.tile(bc, (1, FC // 128)))).astype(BF16)
                acc = acc + _dot_nt(wout[:, c * FC:(c + 1) * FC], h)
            x32[i] = acc

            @pl.when(l == 1)
            def _():
                xio[:, rows] = acc.astype(BF16)
                cp(6 + i, xio.at[:, rows], o_hbm.at[:, rows]).start()

        with jax.named_scope("p2"):
            lax.fori_loop(0, NB, phase2, None)

    lax.fori_loop(0, 2, layer, None)
    for i in range(NB):
        rows = pl.ds(i * TM, TM)
        cp(6 + i, xio.at[:, rows], o_hbm.at[:, rows]).wait()


@jax.jit
def pallas_interleave_layers__sliding_local_dilated__mixer_gmlp__prompt_kernel(
    A_x, A_wqkv, A_wo, B_x, B_w_in, B_w_sp, B_b_sp, B_w_out,
):
    del B_x
    hbm = pl.BlockSpec(memory_space=pltpu.HBM)
    out = pl.pallas_call(
        _kernel,
        in_specs=[hbm, hbm, hbm, hbm, hbm, pl.BlockSpec(memory_space=pltpu.VMEM), hbm],
        out_specs=hbm,
        out_shape=jax.ShapeDtypeStruct((D, S), BF16),
        scratch_shapes=[
            pltpu.VMEM((D, S), BF16), pltpu.VMEM((NB, D, TM), F32),
            pltpu.VMEM((D, 3 * D), BF16), pltpu.VMEM((1792, D), BF16),
            pltpu.VMEM((D, D), BF16), pltpu.VMEM((D, 640), BF16),
            pltpu.VMEM((D, 2 * FH), BF16), pltpu.VMEM((S, S), BF16), pltpu.VMEM((D, FH), BF16),
            pltpu.VMEM((S, FH), BF16), pltpu.VMEM((NB, TM, D), BF16),
            pltpu.VMEM((14, S + HALO, 128), F32), pltpu.VMEM((S, 128), F32),
            pltpu.VMEM((5, 1792, 128), F32), pltpu.VMEM((2, TM, 640), BF16), pltpu.VMEM((2, TM, FH), F32),
            pltpu.VMEM((NB, TM, FH), F32),
            pltpu.SemaphoreType.DMA((6 + NB,)),
        ],
        compiler_params=pltpu.CompilerParams(vmem_limit_bytes=112 * 1024 * 1024),
    )(A_x.reshape(S, D).T, A_wqkv, A_wo, B_w_in, B_w_sp, B_b_sp.reshape(1, S), B_w_out.T)
    return out.T.reshape(1, S, D)
```
